```python
import os as _os
_os.environ.setdefault("JAX_PLATFORMS", "cpu")
import jax
import jax.numpy as jnp

def _softmax(x, axis=-1):
    return jax.nn.softmax(x, axis=axis)
def _gelu(x):
    return jax.nn.gelu(x, approximate=True)
def _silu(x):
    return jax.nn.silu(x)
def _sigmoid(x):
    return jax.nn.sigmoid(x)
def _layernorm(x, axis=-1, eps=1e-5):
    m = jnp.mean(x, axis=axis, keepdims=True)
    v = jnp.var(x, axis=axis, keepdims=True)
    return (x - m) / jnp.sqrt(v + eps)
def _scatter_add(tgt, idx, src, axis=0):
    return tgt.at[idx].add(src)
def _segment_sum(src, seg, n):
    return jax.ops.segment_sum(src, seg, n)
class _Rng:
    def __init__(self, key):
        self._k = key
    def _next(self):
        self._k, sub = jax.random.split(self._k)
        return sub
    def normal(self, shape):
        return jax.random.normal(self._next(), shape, dtype=jnp.bfloat16)
    def randint(self, lo, hi, shape):
        return jax.random.randint(self._next(), shape, lo, hi, dtype=jnp.int32)
    def uniform(self, shape, lo=0.0, hi=1.0):
        return jax.random.uniform(self._next(), shape, jnp.bfloat16, lo, hi)
    def permutation(self, n):
        return jax.random.permutation(self._next(), n)


kernel_name = 'concat_heads__gqa_block_cached__sliding_block_cached__decode'

def setup_inputs():
    _rng = _Rng(jax.random.key(int.from_bytes(__import__("os").urandom(4), "little")))
    _w = (lambda a: (lambda t: t.astype(jnp.bfloat16) if jnp.issubdtype(t.dtype, jnp.floating) else t)(jnp.asarray(a)))
    def _A_setup():
        B, Sq, D = 1, 1, 576
        Hq, Hkv, Sk, Dh = 32, 16, 8192, 128
        assert Hq % Hkv == 0, (Hq, Hkv)
        return {
            "x": _w((lambda *s: _rng.normal(s) * 0.8)(B, Sq, D)),
            "k_cache": _w((lambda *s: _rng.normal(s) * 0.8)(B, Hkv, Sk, Dh)),
            "v_cache": _w((lambda *s: _rng.normal(s) * 0.05)(B, Hkv, Sk, Dh)),
            "wq": _w((lambda *s: _rng.normal(s) * 0.8)(D, Hq * Dh) * (D ** -0.5)),
            "wo": _w((lambda *s: _rng.normal(s) * 0.05)(Hq * Dh, D) * ((Hq * Dh) ** -0.5)),
        }
    _A_in = _A_setup()

    def _B_setup():
        B, Sq, D = 1, 1, 576
        Hq, Hkv, Sk, Dh = 32, 16, 8192, 128
        assert Hq % Hkv == 0, (Hq, Hkv)
        return {
            "x": _w((lambda *s: _rng.normal(s) * 0.8)(B, Sq, D)),
            "k_cache": _w((lambda *s: _rng.normal(s) * 0.8)(B, Hkv, Sk, Dh)),
            "v_cache": _w((lambda *s: _rng.normal(s) * 0.05)(B, Hkv, Sk, Dh)),
            "wq": _w((lambda *s: _rng.normal(s) * 0.8)(D, Hq * Dh) * (D ** -0.5)),
            "wo": _w((lambda *s: _rng.normal(s) * 0.05)(Hq * Dh, D) * ((Hq * Dh) ** -0.5)),
        }
    _B_in = _B_setup()

    return {
        "A_x": _A_in["x"],
        "A_k_cache": _A_in["k_cache"],
        "A_v_cache": _A_in["v_cache"],
        "A_wq": _A_in["wq"],
        "A_wo": _A_in["wo"],
        "B_x": _B_in["x"],
        "B_k_cache": _B_in["k_cache"],
        "B_v_cache": _B_in["v_cache"],
        "B_wq": _B_in["wq"],
        "B_wo": _B_in["wo"],
    }

def reference(A_x, A_k_cache, A_v_cache, A_wq, A_wo, B_x, B_k_cache, B_v_cache, B_wq, B_wo):
    def _A_ref(x, k_cache, v_cache, wq, wo):
        B, Sq, D = x.shape
        Hq, Dh = 32, 128
        Hkv = k_cache.shape[1]
        rep = Hq // Hkv
        q = (lambda x, *d: x.transpose(*d))((x @ wq).reshape(B, Sq, Hq, Dh), 0, 2, 1, 3)
        k = jnp.repeat(k_cache, rep, axis=1)
        v = jnp.repeat(v_cache, rep, axis=1)
        scores = jnp.einsum("bhqd,bhkd->bhqk", q, k) * (Dh ** -0.5)
        p = _softmax(scores, axis=-1)
        o = jnp.einsum("bhqk,bhkd->bhqd", p, v)
        return (lambda x, *d: x.transpose(*d))(o, 0, 2, 1, 3).reshape(B, Sq, Hq * Dh) @ wo

    def _B_ref(x, k_cache, v_cache, wq, wo):
        B, Sq, D = x.shape
        Hq, Dh = 32, 128
        Hkv, Sk = k_cache.shape[1], k_cache.shape[2]
        W = min(4096, max(256, Sk // 4))
        rep = Hq // Hkv
        q = (lambda x, *d: x.transpose(*d))((x @ wq).reshape(B, Sq, Hq, Dh), 0, 2, 1, 3)
        k = jnp.repeat(k_cache[:, :, Sk - W:, :], rep, axis=1)
        v = jnp.repeat(v_cache[:, :, Sk - W:, :], rep, axis=1)
        scores = jnp.einsum("bhqd,bhkd->bhqk", q, k) * (Dh ** -0.5)
        p = _softmax(scores, axis=-1)
        o = jnp.einsum("bhqk,bhkd->bhqd", p, v)
        return (lambda x, *d: x.transpose(*d))(o, 0, 2, 1, 3).reshape(B, Sq, Hq * Dh) @ wo

    a = _A_ref(A_x, A_k_cache, A_v_cache, A_wq, A_wo)
    b = _B_ref(B_x, B_k_cache, B_v_cache, B_wq, B_wo)
    return jnp.concatenate([a, b], axis=-1)
```

```python
import functools
import math

import jax
import jax.numpy as jnp
from jax import lax
from jax.experimental import pallas as pl
from jax.experimental.pallas import tpu as pltpu

D_MODEL = 576
HQ, HKV, DH = 32, 16, 128
BK = 128
F32, BF16 = jnp.float32, jnp.bfloat16
NT = (((1,), (1,)), ((), ()))
NN = (((1,), (0,)), ((), ()))


def make(depth=7, pattern=((1, 1), (1, 0)), interleave=True, nosem=True, nobc=True, flags=None,
         compute=True, nslot=None):
    per = sum(m for m, _ in pattern)
    assert 16 % per == 0 and (per <= 8)
    nsub = 16 // per

    def kern(xa, ka, va, wqa, woa, xb, kb, vb, wqb, wob, out,
             x_v, wq_v, kv_v, wo_v, q_v, s_v, o_v, out_v, sems, xsem, osem):
        sk = ka.shape[2]
        win = min(4096, max(256, sk // 4))
        na, nb = sk // BK, win // BK
        nkv = na + nb
        ring = kv_v.shape[0]

        def w_issue(src, dst):
            def f(j, u, sem):
                r = j * 8 if isinstance(j, int) else pl.multiple_of(j * 8, 8)
                g = u * per
                for m, p in pattern:
                    c, g8 = divmod(g, 8)
                    idx = (pl.ds(g8, m), pl.ds(r, 8), pl.ds(c * 2048, 2048))
                    pltpu.make_async_copy(src.at[idx], dst.at[idx], sem).start(priority=p)
                    g += m
            return f

        def kv_issue(src, row0, slot0):
            def f(j, u, sem):
                r = row0 + j * BK
                if not isinstance(r, int):
                    r = pl.multiple_of(r, BK)
                slot = (slot0 + j) % ring
                g = u * per
                for m, p in pattern:
                    pltpu.make_async_copy(src.at[0, pl.ds(g, m), pl.ds(r, BK)],
                                          kv_v.at[slot, pl.ds(g, m)], sem).start(priority=p)
                    g += m
            return f

        phases = [(9, w_issue(wqa, wq_v.at[0])), (9, w_issue(wqb, wq_v.at[1])),
                  (na, kv_issue(ka, 0, 0)), (nb, kv_issue(kb, sk - win, na)),
                  (na, kv_issue(va, 0, nkv)), (nb, kv_issue(vb, sk - win, nkv + na)),
                  (9, w_issue(woa, wo_v.at[0])), (9, w_issue(wob, wo_v.at[1]))]
        starts = [0]
        for n, _ in phases:
            starts.append(starts[-1] + n)
        total = starts[-1]

        def phase_of(i):
            for p in range(len(phases)):
                if starts[p] <= i < starts[p + 1]:
                    return p
            return None

        def wait(i):
            pltpu.make_async_copy(kv_v.at[0], kv_v.at[0], sems.at[i % depth]).wait()

        def run(lo, hi, body, carry):
            i = lo
            while i < hi:
                p = phase_of(i + depth)
                j = i
                while j < hi and phase_of(j + depth) == p:
                    j += 1

                def step(t, c, p=p):
                    wait(t)
                    state = [0]

                    def tick(frac):
                        while p is not None and state[0] < nsub and (state[0] <= frac * nsub or not interleave):
                            phases[p][1](t + depth - starts[p], state[0], sems.at[t % depth])
                            state[0] += 1
                    if compute:
                        c = body(t - lo, tick, c)
                    tick(1.0)
                    return c
                carry = lax.fori_loop(i, j, step, carry)
                i = j
            return carry

        for i in range(depth):
            p = phase_of(i)
            for u in range(nsub):
                phases[p][1](i - starts[p], u, sems.at[i])
            if i == 0:
                cx = [pltpu.make_async_copy(xa, x_v.at[0], xsem.at[0]),
                      pltpu.make_async_copy(xb, x_v.at[1], xsem.at[1])]
                for c in cx:
                    c.start()

        row = lax.broadcasted_iota(jnp.int32, (8, 128), 0)

        run(0, 9, lambda j, tick, c: c, 0)
        for c in cx:
            c.wait()

        def q_body(j, tick, c):
            br, cb = j // 8, j % 8
            x = jnp.broadcast_to(x_v[br, 0].astype(F32), (8, D_MODEL)).astype(BF16)
            qs = None
            for t in range(4):
                tick(t / 4)
                col = pl.multiple_of(cb * 512 + t * 128, 128)
                w = wq_v[br, :, :, pl.ds(col, 128)].reshape(D_MODEL, 128)
                r = lax.dot_general(x, w, NN, preferred_element_type=F32)
                qs = r if qs is None else jnp.where(row % 4 == t, r, qs)
            q_v[pl.ds(j * 4, 4), :] = qs[:4]
            return c
        run(9, 25, q_body, 0)

        def s_body(off, br):
            def f(j, tick, ms):
                jj = off + j
                slot = jj % ring
                new = []
                for g in range(4):
                    q = q_v[pl.ds(br * HQ + g * 8, 8), :].astype(BF16)
                    s = None
                    for h in range(4):
                        tick((g * 4 + h) / 16)
                        r = lax.dot_general(q, kv_v[slot, g * 4 + h], NT, preferred_element_type=F32)
                        s = r if s is None else jnp.where(row // 2 == h, r, s)
                    s_v[jj, g] = s
                    new.append(jnp.maximum(ms[g], s))
                return tuple(new)
            return f
        ninf = tuple(jnp.full((8, 128), -jnp.inf, F32) for _ in range(4))
        m_a = run(25, 25 + na, s_body(0, 0), ninf)
        m_b = run(25 + na, 25 + nkv, s_body(na, 1), ninf)
        mx = [[jnp.broadcast_to(jnp.max(m, axis=1, keepdims=True), (8, 128)) for m in ms] for ms in (m_a, m_b)]

        scale = (DH ** -0.5) * math.log2(math.e)

        def pv_body(off, br):
            def f(j, tick, c):
                ls, accs = c
                jj = off + j
                slot = (nkv + jj) % ring
                nl, nacc = [], []
                for g in range(4):
                    p = jnp.exp2((s_v[jj, g] - mx[br][g]) * scale)
                    nl.append(ls[g] + p)
                    pb = p.astype(BF16)
                    o = None
                    for h in range(4):
                        tick((g * 4 + h) / 16)
                        r = lax.dot_general(pb, kv_v[slot, g * 4 + h], NN, preferred_element_type=F32)
                        o = r if o is None else jnp.where(row // 2 == h, r, o)
                    nacc.append(accs[g] + o)
                return tuple(nl), tuple(nacc)
            return f
        zero = tuple(jnp.zeros((8, 128), F32) for _ in range(4))
        t0 = 25 + nkv
        for br, (lo, n, off) in enumerate(((t0, na, 0), (t0 + na, nb, na))):
            ls, accs = run(lo, lo + n, pv_body(off, br), (zero, zero))
            for g in range(4):
                o_v[pl.ds(br * HQ + g * 8, 8), :] = accs[g] / jnp.sum(ls[g], axis=1, keepdims=True)

        t0 = 25 + 2 * nkv
        run(t0, total - 9, lambda j, tick, c: c, 0)

        def o_body(br):
            def f(j, tick, acc):
                for t in range(4):
                    tick(t / 4)
                    h = j * 4 + t
                    o = jnp.broadcast_to(o_v[pl.ds(br * HQ + h, 1), :], (8, 128)).astype(BF16)
                    col = pl.multiple_of(h * 128, 128)
                    w = wo_v[br, :, :, pl.ds(col, 128)].reshape(D_MODEL, 128)
                    acc = acc + lax.dot_general(o, w, NT, preferred_element_type=F32)
                return acc
            return f
        z = jnp.zeros((8, D_MODEL), F32)
        ra = run(total - 9, total - 1, o_body(0), z)
        wait(total - 1)
        rb = z
        if compute:
            rb = lax.fori_loop(0, 8, lambda j, c: o_body(1)(j, lambda f: None, c), z)
        out_v[0] = jnp.concatenate([ra[:1], rb[:1]], axis=1).astype(BF16)
        c = pltpu.make_async_copy(out_v, out, osem)
        c.start()
        c.wait()

    def fn(A_x, A_k_cache, A_v_cache, A_wq, A_wo, B_x, B_k_cache, B_v_cache, B_wq, B_wo):
        hbm = pl.BlockSpec(memory_space=pltpu.HBM)
        wv = (8, 72, 4096)
        ring = nslot or 160
        return pl.pallas_call(
            kern,
            out_shape=jax.ShapeDtypeStruct((1, 1, 2 * D_MODEL), BF16),
            in_specs=[hbm] * 10, out_specs=hbm,
            scratch_shapes=[
                pltpu.VMEM((2, 1, 1, D_MODEL), BF16),
                pltpu.VMEM((2,) + wv, BF16),
                pltpu.VMEM((ring, HKV, BK, DH), BF16),
                pltpu.VMEM((2,) + wv, BF16),
                pltpu.VMEM((2 * HQ, DH), F32),
                pltpu.VMEM((80, 4, 8, BK), F32),
                pltpu.VMEM((2 * HQ, DH), F32),
                pltpu.VMEM((1, 1, 2 * D_MODEL), BF16),
                pltpu.SemaphoreType.DMA((depth,)),
                pltpu.SemaphoreType.DMA((2,)),
                pltpu.SemaphoreType.DMA(()),
            ],
            compiler_params=pltpu.CompilerParams(
                vmem_limit_bytes=120 * 2**20, disable_bounds_checks=nobc,
                disable_semaphore_checks=nosem, flags=flags),
        )(A_x, A_k_cache, A_v_cache, A_wq.reshape(wv), A_wo.T.reshape(wv),
          B_x, B_k_cache, B_v_cache, B_wq.reshape(wv), B_wo.T.reshape(wv))
    return fn


@jax.jit
def pallas_concat_heads__gqa_block_cached__sliding_block_cached__decode_kernel(
        A_x, A_k_cache, A_v_cache, A_wq, A_wo, B_x, B_k_cache, B_v_cache, B_wq, B_wo):
    return make()(A_x, A_k_cache, A_v_cache, A_wq, A_wo, B_x, B_k_cache, B_v_cache, B_wq, B_wo)
```

```python
import math

import jax
import jax.numpy as jnp
from jax import lax
from jax.experimental import pallas as pl
from jax.experimental.pallas import tpu as pltpu

DM = 576
HQ, HKV, DH = 32, 16, 128
HD = HQ * DH
HALF = HD // 2
GROUPS = HQ // 8
BK = 128
WB, WR = 9, 64
WSTEPS = WR // 8
DEPTH = 6
RING = 8
PREFILL = 24
LAST_COLS = (1024, 512, 512)

F32, BF16 = jnp.float32, jnp.bfloat16
NN = (((1,), (0,)), ((), ()))
NT = (((1,), (1,)), ((), ()))


def _window(sk):
    return min(4096, max(256, sk // 4))


def _ds(start, size, align):
    return pl.ds(start if isinstance(start, int) else pl.multiple_of(start, align), size)


def _wait_filled(buf, sem):
    pltpu.make_async_copy(buf, buf, sem).wait()


def _kernel(xa, ka, va, wqa, woa, xb, kb, vb, wqb, wob, out,
            x_v, wq_v, kv_v, wo_v, q_v, s_v, o_v, out_v, sems, tail_sems, io_sem):
    sk_b = kb.shape[2]
    win = _window(sk_b)
    na, nb = ka.shape[2] // BK, win // BK
    nkv = na + nb

    def weight_phase(src, dst, block0):
        def issue(j, sem, n_low=0):
            for u in range(16):
                b, m = ((0, 8), (8, 1))[u % 2]
                rows, cols = _ds(j * 8, 8, 8), pl.ds(u // 2 * 512, 512)
                pltpu.make_async_copy(
                    src.at[pl.ds(b, m), rows, cols], dst.at[pl.ds(block0 + b, m), rows, cols], sem
                ).start(priority=1 if u < n_low else 1 - u % 2)
        return WSTEPS, issue, lambda j: dst.at[pl.ds(block0, WB), _ds(j * 8, 8, 8)]

    def cache_phase(src, row0, n, slot0):
        def issue(j, sem):
            for u in range(16):
                r = u // 8 * 64
                h, m = ((0, 3), (3, 1))[u % 2]
                heads = pl.ds(u % 8 // 2 * 4 + h, m)
                pltpu.make_async_copy(
                    src.at[0, heads, _ds(row0 + j * BK + r, 64, 64)],
                    kv_v.at[(slot0 + j) % RING, heads, pl.ds(r, 64)], sem
                ).start(priority=1 - u % 2)
        return n, issue, lambda j: kv_v.at[(slot0 + j) % RING]

    def start_woa(block0, n_blocks, row, col, n_cols, k, priority):
        idx = (pl.ds(block0, n_blocks), _ds(row, 8, 8), pl.ds(col, n_cols))
        pltpu.make_async_copy(woa.at[idx], wo_v.at[idx], tail_sems.at[k]).start(priority=priority)

    def woa_phase(col0, parts):
        def issue(j, sem):
            for u in range(16):
                b, m, k = parts[u % 2]
                start_woa(b, m, j * 16 + u // 8 * 8, col0 + u % 8 // 2 * 512, 512, k, 1 - u % 2)
        return WSTEPS // 2, issue, None

    phases = [weight_phase(wqb, wq_v, WB), weight_phase(wqa, wq_v, 0), weight_phase(wob, wo_v, WB),
              cache_phase(kb, sk_b - win, nb, 0), cache_phase(ka, 0, na, nb),
              cache_phase(vb, sk_b - win, nb, nkv), cache_phase(va, 0, na, nkv + nb),
              woa_phase(0, ((0, 8, 0), (8, 1, 0))), woa_phase(HALF, ((0, 4, 1), (8, 1, 2)))]
    steps = [(phase, j) for phase in phases for j in range(phase[0])]
    consumed = 0

    def consume(n, body, carry):
        nonlocal consumed
        first = consumed
        while consumed < first + n:
            i = consumed
            (cur, jc), (nxt, jn) = steps[i], steps[i + DEPTH]

            def step(t, c, i=i, cur=cur, jc=jc, nxt=nxt, jn=jn):
                _wait_filled(cur[2](jc + t), sems.at[(i + t) % RING])
                nxt[1](jn + t, sems.at[(i + t + DEPTH) % RING])
                return body(i - first + t, c)
            count = min(first + n - i, cur[0] - jc, nxt[0] - jn)
            carry = lax.fori_loop(0, count, step, carry)
            consumed += count
        return carry

    n_prefill = pl.cdiv(PREFILL, 16)
    for i in range(n_prefill):
        phases[0][1](i, sems.at[i], PREFILL - 16 * i)
    pltpu.make_async_copy(xa, x_v.at[0], io_sem).start()
    pltpu.make_async_copy(xb, x_v.at[1], io_sem).start()
    lax.fori_loop(n_prefill, DEPTH, lambda i, c: phases[0][1](i, sems.at[i]), None)

    row = lax.broadcasted_iota(jnp.int32, (8, 128), 0)
    lane = lax.broadcasted_iota(jnp.int32, (1, 128), 1)

    def q_body(br):
        def body(j, c):
            x = jnp.broadcast_to(x_v[br, 0].astype(F32), (8, DM)).astype(BF16)
            w = wq_v[pl.ds(br * WB, WB), :, _ds(j * 512, 512, 512)].reshape(DM, 512)
            q = lax.dot_general(x, w, NN, preferred_element_type=F32)
            for t in range(4):
                q_v[pl.ds(br * HQ + j * 4 + t, 1), :] = q[:1, t * DH:(t + 1) * DH]
            return c
        return body

    consume(WSTEPS, lambda j, c: c, None)
    _wait_filled(x_v, io_sem)
    consume(WSTEPS, q_body(1), None)
    consume(WSTEPS, q_body(0), None)

    def group_dot(lhs, slot, g, dims):
        res = None
        for h in range(4):
            r = lax.dot_general(lhs, kv_v[slot, g * 4 + h], dims, preferred_element_type=F32)
            res = r if res is None else jnp.where(row >= 2 * h, r, res)
        return res

    def score_body(br, off):
        def body(j, maxes):
            new = []
            for g in range(GROUPS):
                q = q_v[pl.ds(br * HQ + g * 8, 8), :].astype(BF16)
                s = group_dot(q, (off + j) % RING, g, NT)
                s_v[off + j, g] = s
                new.append(jnp.maximum(maxes[g], s))
            return tuple(new)
        return body

    neg_inf = (jnp.full((8, BK), -jnp.inf, F32),) * GROUPS
    max_b = consume(nb, score_body(1, 0), neg_inf)
    max_a = consume(na, score_body(0, nb), neg_inf)
    row_max = [[jnp.broadcast_to(jnp.max(m, axis=1, keepdims=True), (8, BK)) for m in maxes]
               for maxes in (max_a, max_b)]

    scale = DH ** -0.5 * math.log2(math.e)

    def pv_body(br, off):
        def body(j, c):
            sums, accs = [], []
            for g in range(GROUPS):
                p = jnp.exp2((s_v[off + j, g] - row_max[br][g]) * scale)
                sums.append(c[0][g] + p)
                accs.append(c[1][g] + group_dot(p.astype(BF16), (nkv + off + j) % RING, g, NN))
            return tuple(sums), tuple(accs)
        return body

    def normalize(br, c):
        for g in range(GROUPS):
            o_v[pl.ds(br * HQ + g * 8, 8), :] = c[1][g] / jnp.sum(c[0][g], axis=1, keepdims=True)

    def project(br, block0, n_blocks, h0, n_heads, acc):
        for t in range(n_heads):
            h = h0 + t
            head = lambda b: jnp.broadcast_to(o_v[pl.ds(b * HQ + h, 1), :], (8, DH))
            o = jnp.where(row == 0, head(0), head(1)) if br is None else head(br)
            w = wo_v[pl.ds(block0, n_blocks), :, _ds(h * DH, DH, DH)].reshape(n_blocks * WR, DH)
            acc = acc + lax.dot_general(o.astype(BF16), w, NT, preferred_element_type=F32)
        return acc

    def woa_landed(k, block0, n_blocks, col, n_cols):
        _wait_filled(wo_v.at[pl.ds(block0, n_blocks), :, pl.ds(col, n_cols)], tail_sems.at[k])

    zeros = ((jnp.zeros((8, DH), F32),) * GROUPS,) * 2
    normalize(1, consume(nb, pv_body(1, 0), zeros))
    pv_a, out_b = consume(
        8, lambda j, c: (pv_body(0, nb)(j, c[0]), project(1, WB + 1, WB - 1, j * 4, 4, c[1])),
        (zeros, jnp.zeros((8, 512), F32)))
    out_v[0, :, 640:] = out_b[:1].astype(BF16)
    normalize(0, consume(na - 8, pv_body(0, nb + 8), pv_a))

    for phase, j in steps[consumed + DEPTH:]:
        phase[1](j, None)
    for r in range(0, WR, 8):
        start_woa(4, 2, r, HALF, HALF, 3, 1)
    last = [(HALF + sum(LAST_COLS[:i]), n) for i, n in enumerate(LAST_COLS)]
    for i, (col, n) in enumerate(last):
        for r in range(0, WR, 8):
            start_woa(6, 2, r, col, n, 4 + i, 1)

    woa_landed(0, 0, WB, 0, HALF)
    acc = lax.fori_loop(0, 2, lambda i, a: project(None, 0, WB + 1, i * 8, 8, a),
                        jnp.zeros((8, 640), F32))
    woa_landed(2, 8, 1, HALF, HALF)
    both = project(None, 8, 2, 16, 16, acc[:, 512:])
    out_v[0, :, 512:640] = jnp.where(lane < WR, both[0:1], both[1:2]).astype(BF16)
    woa_landed(1, 0, 4, HALF, HALF)
    out_v[0, :, :256] = project(0, 0, 4, 16, 16, acc[:, :256])[:1].astype(BF16)
    woa_landed(3, 4, 2, HALF, HALF)
    out_v[0, :, 256:384] = project(0, 4, 2, 16, 16, acc[:, 256:384])[:1].astype(BF16)
    acc = acc[:, 384:512]
    for i, (col, n) in enumerate(last):
        woa_landed(4 + i, 6, 2, col, n)
        acc = project(0, 6, 2, col // DH, n // DH, acc)
    out_v[0, :, 384:512] = acc[:1].astype(BF16)

    write = pltpu.make_async_copy(out_v, out, io_sem)
    write.start()
    write.wait()


@jax.jit
def pallas_concat_heads__gqa_block_cached__sliding_block_cached__decode_kernel(
    A_x: jax.Array,
    A_k_cache: jax.Array,
    A_v_cache: jax.Array,
    A_wq: jax.Array,
    A_wo: jax.Array,
    B_x: jax.Array,
    B_k_cache: jax.Array,
    B_v_cache: jax.Array,
    B_wq: jax.Array,
    B_wo: jax.Array,
):
    sk_a, sk_b = A_k_cache.shape[2], B_k_cache.shape[2]
    win = _window(sk_b)
    assert A_x.shape == B_x.shape == (1, 1, DM)
    assert A_k_cache.shape == A_v_cache.shape == (1, HKV, sk_a, DH)
    assert B_k_cache.shape == B_v_cache.shape == (1, HKV, sk_b, DH)
    assert sk_a % BK == 0 and sk_a >= 8 * BK and sk_b % BK == 0 and win % BK == 0 and win <= sk_b

    hbm = pl.BlockSpec(memory_space=pltpu.HBM)
    blocks = (WB, WR, HD)
    return pl.pallas_call(
        _kernel,
        out_shape=jax.ShapeDtypeStruct((1, 1, 2 * DM), BF16),
        in_specs=[hbm] * 10,
        out_specs=hbm,
        scratch_shapes=[
            pltpu.VMEM((2, 1, 1, DM), BF16),
            pltpu.VMEM((2 * WB, WR, HD), BF16),
            pltpu.VMEM((RING, HKV, BK, DH), BF16),
            pltpu.VMEM((2 * WB, WR, HD), BF16),
            pltpu.VMEM((2 * HQ, DH), F32),
            pltpu.VMEM(((sk_a + win) // BK, GROUPS, 8, BK), F32),
            pltpu.VMEM((2 * HQ, DH), F32),
            pltpu.VMEM((1, 1, 2 * DM), BF16),
            pltpu.SemaphoreType.DMA((RING,)),
            pltpu.SemaphoreType.DMA((4 + len(LAST_COLS),)),
            pltpu.SemaphoreType.DMA(()),
        ],
        compiler_params=pltpu.CompilerParams(
            vmem_limit_bytes=48 * 2**20, disable_semaphore_checks=True),
    )(
        A_x, A_k_cache, A_v_cache, A_wq.reshape(blocks), A_wo.T.reshape(blocks),
        B_x, B_k_cache, B_v_cache, B_wq.reshape(blocks), B_wo.T.reshape(blocks),
    )
```
